```python
import jax
import jax.numpy as jnp

def _softmax(x, axis=-1):
    return jax.nn.softmax(x, axis=axis)

def _gelu(x):
    return jax.nn.gelu(x, approximate=True)

def _silu(x):
    return jax.nn.silu(x)

def _sigmoid(x):
    return jax.nn.sigmoid(x)

def _layernorm(x, axis=-1, eps=1e-05):
    m = jnp.mean(x, axis=axis, keepdims=True)
    v = jnp.var(x, axis=axis, keepdims=True)
    return (x - m) / jnp.sqrt(v + eps)

def _scatter_add(tgt, idx, src, axis=0):
    return tgt.at[idx].add(src)

def _segment_sum(src, seg, n):
    return jax.ops.segment_sum(src, seg, n)

class _Rng:

    def __init__(self, key):
        self._k = key

    def _next(self):
        self._k, sub = jax.random.split(self._k)
        return sub

    def normal(self, shape):
        return jax.random.normal(self._next(), shape, dtype=jnp.bfloat16)

    def randint(self, lo, hi, shape):
        return jax.random.randint(self._next(), shape, lo, hi, dtype=jnp.int32)

    def uniform(self, shape, lo=0.0, hi=1.0):
        return jax.random.uniform(self._next(), shape, jnp.bfloat16, lo, hi)

    def permutation(self, n):
        return jax.random.permutation(self._next(), n)
kernel_name = 'adaLN_cond__mha_block_cached__moe_arch_mod__prompt'

def setup_inputs():
    _rng = _Rng(jax.random.key(int.from_bytes(__import__("os").urandom(4), "little")))
    _w = lambda a: (lambda t: t.astype(jnp.bfloat16) if jnp.issubdtype(t.dtype, jnp.floating) else t)(jnp.asarray(a))

    def _A_setup():
        B, Sq, D = (1, 2048, 1024)
        H, Sk, Dh = (32, 2048, 128)
        return {'x': _w((lambda *s: _rng.normal(s) * 0.05)(B, Sq, D)), 'k_cache': _w((lambda *s: _rng.normal(s) * 0.05)(B, H, Sk, Dh)), 'v_cache': _w((lambda *s: _rng.normal(s) * 0.05)(B, H, Sk, Dh)), 'wq': _w((lambda *s: _rng.normal(s) * 0.05)(D, H * Dh) * D ** (-0.5)), 'wo': _w((lambda *s: _rng.normal(s) * 0.05)(H * Dh, D) * (H * Dh) ** (-0.5))}
    _A_in = _A_setup()

    def _B_setup():
        B, S, D, F, C = (1, 2048, 1024, 3584, 2)
        return {'x': _w((lambda *s: _rng.normal(s) * 0.05)(B, S, D)), 'w_r': _w((lambda *s: _rng.normal(s) * 0.05)(D)), 'w_gate': _w((lambda *s: _rng.normal(s) * 0.05)(D, F)), 'w_up': _w((lambda *s: _rng.normal(s) * 0.05)(D, F)), 'w_down': _w((lambda *s: _rng.normal(s) * 0.05)(F, D))}
    _B_in = _B_setup()
    return {'A_x': _A_in['x'], 'A_k_cache': _A_in['k_cache'], 'A_v_cache': _A_in['v_cache'], 'A_wq': _A_in['wq'], 'A_wo': _A_in['wo'], 'B_x': _B_in['x'], 'B_w_r': _B_in['w_r'], 'B_w_gate': _B_in['w_gate'], 'B_w_up': _B_in['w_up'], 'B_w_down': _B_in['w_down'], 'c': _w((lambda *s: _rng.normal(s) * 0.05)(1, 1024)), 'w_mod': _w((lambda *s: _rng.normal(s) * 0.05)(1024, 6 * 1024) * 1024 ** (-0.5))}

def reference(A_x, A_k_cache, A_v_cache, A_wq, A_wo, B_x, B_w_r, B_w_gate, B_w_up, B_w_down, c, w_mod):

    def _A_ref(x, k_cache, v_cache, wq, wo):
        B, Sq, D = x.shape
        H, Dh = (32, 128)
        q = (lambda x, *d: x.transpose(*d))((x @ wq).reshape(B, Sq, H, Dh), 0, 2, 1, 3)
        scores = jnp.einsum('bhqd,bhkd->bhqk', q, k_cache) * Dh ** (-0.5)
        p = _softmax(scores, axis=-1)
        o = jnp.einsum('bhqk,bhkd->bhqd', p, v_cache)
        return (lambda x, *d: x.transpose(*d))(o, 0, 2, 1, 3).reshape(B, Sq, H * Dh) @ wo

    def _B_ref(x, w_r, w_gate, w_up, w_down):
        B, S, D = x.shape
        C = 2
        r = x @ w_r
        idx = jnp.argsort(-r, axis=-1)[:, :C]
        idx_e = jnp.repeat(idx.reshape(B, C, 1), D, axis=2)
        x_sel = jnp.take_along_axis(x, idx_e, axis=1)
        g = _silu(x_sel @ w_gate)
        u = x_sel @ w_up
        y = g * u @ w_down
        r_sel = _sigmoid(jnp.take_along_axis(r, idx, axis=1))
        y = y * r_sel.reshape(B, C, 1)
        b_off = (jnp.arange(B) * S).reshape(B, 1)
        flat_idx = (idx + b_off).reshape(B * C)
        zero = (x * 0.0).reshape(B * S, D)
        upd = _scatter_add(zero, flat_idx, y.reshape(B * C, D), axis=0)
        return x + upd.reshape(B, S, D)
    x = A_x
    mod = (_silu(c) @ w_mod).reshape(c.shape[0], 6, 1, -1)
    sa, ca, ga, sb, cb, gb = (mod[:, 0].copy(), mod[:, 1].copy(), mod[:, 2].copy(), mod[:, 3].copy(), mod[:, 4].copy(), mod[:, 5].copy())
    h = _layernorm(x, axis=-1) * (1 + ca) + sa
    x = x + ga * _A_ref(h, A_k_cache, A_v_cache, A_wq, A_wo)
    h = _layernorm(x, axis=-1) * (1 + cb) + sb
    x = x + gb * _B_ref(h, B_w_r, B_w_gate, B_w_up, B_w_down)
    return x
```

```python
import numpy as np
import jax
import jax.numpy as jnp
from jax import lax
import jax.experimental.pallas as pl
import jax.experimental.pallas.tpu as pltpu

S = 2048
D = 1024
H = 32
DH = 128
F = 3584
EPS = 1e-5
BF = jnp.bfloat16
F32 = jnp.float32
U32 = jnp.uint32
I32 = jnp.int32
LOG2E = 1.4426950408889634
QSCALE = (DH ** -0.5) * LOG2E
NT_DIMS = (((1,), (1,)), ((), ()))
TN_DIMS = (((0,), (0,)), ((), ()))

BQ = 512
NT = S // BQ
NQ = BQ // 128
GROUPS = ((0, 1), (1, 2), (2, 6), (6, H))


def pk(x):
    return pltpu.bitcast(x, U32)


def upk(x):
    return pltpu.bitcast(x, BF)


def ln(xf):
    mu = jnp.mean(xf, axis=-1, keepdims=True)
    xc = xf - mu
    var = jnp.mean(xc * xc, axis=-1, keepdims=True)
    return xc * lax.rsqrt(var + EPS)


def build(KG=512, LC=64, PACKW=True, MODH=8, QSPLIT=True, PEEL0=True, PEEL1=True, QS=256, EC=64, LG=0, LORD=1, QS1=512, GB=0, GC=0, TQ=1, TREE=0, DL=(1,2,3,4,5,6,7,8), QP=2, NCH=2, UR=16):
    def kernel(x_hbm, k_hbm, v_hbm, wq_hbm, wo_hbm, wr_hbm, wg_hbm, wu_hbm, wd_hbm, c_hbm, wmod_hbm,
               o_hbm,
               xb, hb, kb, vb, wqb, wob, acc, qb, ot, vt, tmp0, tmp1, tmp2, tmp3, mu_b, rs_b,
               wg, wu, wd, wm, cb_, wrb, mod, ob, pb,
               sem_s, sem_x, sem_h, sem_m, sem_w, sem_o):
        def pw(ref):
            return ref.bitcast(BF) if PACKW else ref

        def ldw(val):
            return upk(val) if PACKW else val

        def group_copies(g):
            a, b = GROUPS[g]
            return [pltpu.make_async_copy(wq_hbm.at[:, a * DH:b * DH], pw(wqb).at[:, a * DH:b * DH], sem_h.at[g, 0]),
                    pltpu.make_async_copy(k_hbm.at[a:b], pw(kb).at[a:b], sem_h.at[g, 1]),
                    pltpu.make_async_copy(v_hbm.at[a:b], pw(vb).at[a:b], sem_h.at[g, 2]),
                    pltpu.make_async_copy(wo_hbm.at[a * DH:b * DH, :], pw(wob).at[a * DH:b * DH, :], sem_h.at[g, 3])]

        MC = 512
        cp_c = pltpu.make_async_copy(c_hbm, cb_, sem_s.at[0])
        cp_r = pltpu.make_async_copy(wr_hbm, wrb, sem_s.at[1])
        cp_x = [pltpu.make_async_copy(x_hbm.at[j * BQ:(j + 1) * BQ], xb.at[j * BQ:(j + 1) * BQ], sem_x.at[j])
                for j in range(NT)]
        cp_m = [pltpu.make_async_copy(wmod_hbm.at[:, i * MC:(i + 1) * MC], pw(wm).at[:, i * MC:(i + 1) * MC],
                                      sem_m.at[i]) for i in range(2 * D // MC)]
        cp_m2 = pltpu.make_async_copy(wmod_hbm.at[:, 2 * D:], pw(wm).at[:, 2 * D:], sem_m.at[2 * D // MC])
        cp_w = [pltpu.make_async_copy(wg_hbm, pw(wg), sem_w.at[0]),
                pltpu.make_async_copy(wu_hbm, pw(wu), sem_w.at[1]),
                pltpu.make_async_copy(wd_hbm, pw(wd), sem_w.at[2])]
        cp_o = [pltpu.make_async_copy(ob.bitcast(BF).at[j * BQ:(j + 1) * BQ], o_hbm.at[j * BQ:(j + 1) * BQ], sem_o.at[j])
                for j in range(NT)]
        g0 = group_copies(0)
        g1 = group_copies(1)

        tmp = (tmp0, tmp1, tmp2, tmp3)

        def hrows(j, lo=0, n=BQ):
            return pl.ds((j * BQ + lo) // 2, n // 2)

        def gate(val):
            v = jnp.broadcast_to(val[-8:], (8, 128))
            return jnp.where(v < 0.0, 1, 0).astype(I32)[0, 0]

        def do_ln1(j, z=None):
            chain = []
            for c0 in range(0, BQ, LC):
                r0 = j * BQ + c0
                if LG and len(chain) >= LG:
                    z = chain[-LG]
                if z is not None:
                    r0 = pl.multiple_of(r0 + z * 16, 16)
                xf = xb[pl.ds(r0, LC), :].astype(F32)
                mu = jnp.mean(xf, axis=-1, keepdims=True)
                xc = xf - mu
                rstd = lax.rsqrt(jnp.mean(xc * xc, axis=-1, keepdims=True) + EPS)
                if LG:
                    chain.append(gate(rstd))
                hv = xc * rstd * (1.0 + mod[0:1, D:2 * D]) + mod[0:1, 0:D]
                hb[hrows(j, c0, LC), :] = pk(hv.astype(BF))

        def do_qproj(h, j):
            w = ldw(wqb[:, pl.ds(pl.multiple_of(h * DH, DH), DH)])
            q = jnp.dot(upk(hb[hrows(j), :]), w, preferred_element_type=F32)
            qb[j] = pk((q * QSCALE).astype(BF))

        def do_qk(h, j, mid=None, split=0):
            def part(a, b):
                sl = slice(a // 2, b // 2) if PACKW else slice(a, b)
                return lax.dot_general(ldw(kb[h, sl, :]), upk(qb[j]), NT_DIMS, preferred_element_type=F32)
            if mid is None:
                s = part(0, S)
                return s, jnp.max(s, axis=0, keepdims=True)
            if split == 0:
                mid()
                s = part(0, S)
                return s, jnp.max(s, axis=0, keepdims=True)
            s0 = part(0, split)
            mid()
            s1 = part(split, S)
            s = jnp.concatenate([s0, s1], axis=0)
            return s, jnp.maximum(jnp.max(s0, axis=0, keepdims=True), jnp.max(s1, axis=0, keepdims=True))

        WOR = DH // 2 if PACKW else DH

        def wo_of(h):
            return ldw(wob[pl.ds(pl.multiple_of(h * WOR, WOR), WOR), :])

        def do_oproj(h, j):
            acc[j * BQ:(j + 1) * BQ, :] += lax.dot_general(upk(ot[j]), wo_of(h), TN_DIMS, preferred_element_type=F32)

        def do_oproj_q(h, j, c):
            r = slice(j * BQ + c * 128, j * BQ + (c + 1) * 128)
            acc[r, :] += lax.dot_general(upk(ot[j, :, c * 128:(c + 1) * 128]), wo_of(h), TN_DIMS,
                                         preferred_element_type=F32)

        def do_vt(h, slot):
            for i in range(S // 128):
                if PACKW:
                    vs = upk(vb[h, i * 64:(i + 1) * 64, :])
                else:
                    vs = vb[h, i * 128:(i + 1) * 128, :]
                vt[slot, i] = pk(vs.T)

        def do_pv_q(slot, jj, j, sm):
            s, m = sm
            mj = m[:, j * 128:(j + 1) * 128]
            o = None
            l = None
            for g in range(S // KG):
                p = jnp.exp2(s[g * KG:(g + 1) * KG, j * 128:(j + 1) * 128] - mj)
                if TREE:
                    t = p
                    while t.shape[0] > 8:
                        hf = t.shape[0] // 2
                        t = t[:hf] + t[hf:]
                    l = t if l is None else l + t
                else:
                    ls = jnp.sum(p, axis=0, keepdims=True)
                    l = ls if l is None else l + ls
                lhs = jnp.concatenate([upk(vt[slot, g * (KG // 128) + u]) for u in range(KG // 128)], axis=1)
                d = jnp.dot(lhs, p.astype(BF), preferred_element_type=F32)
                o = d if o is None else o + d
            if TREE:
                l = jnp.sum(l, axis=0, keepdims=True)
            ot[jj, :, j * 128:(j + 1) * 128] = pk((o * (1.0 / l)).astype(BF))
            return l

        def do_pv(slot, jj, m):
            return [do_pv_q(slot, jj, j, m) for j in range(NQ)]

        def epi_consts():
            cb1 = 1.0 + mod[0:1, 4 * D:5 * D]
            sbv = mod[0:1, 3 * D:4 * D]
            gb = mod[0:1, 5 * D:6 * D]
            wr = wrb[...].astype(F32)
            return gb * cb1, gb * sbv, wr * cb1, jnp.sum(wr * sbv, axis=-1, keepdims=True)

        def gated(base, z):
            return base if z is None else pl.multiple_of(base + z * 8, 8)

        pid = gate(jnp.exp2(mod[0:8, 0:128]))

        def epi_a(h, j, lo, n, buf=None):
            rr = slice(j * BQ + lo, j * BQ + lo + n)
            d = lax.dot_general(upk(ot[j, :, lo:lo + n]), wo_of(h), TN_DIMS, preferred_element_type=F32)
            x1 = xb[rr, :].astype(F32) + mod[0:1, 2 * D:3 * D] * (acc[rr, :] + d)
            if buf is None:
                acc[rr, :] = x1
            else:
                buf[...] = x1
            return x1, jnp.broadcast_to(jnp.mean(x1, axis=-1, keepdims=True), (n, 128))

        def epi_bc(r0, n, xv, mu, top, consts, copy, z=None):
            m1, i1, m2, i2 = top
            ca_, cb2, w2, r0c = consts
            xc = xv - (jnp.concatenate([mu] * (D // 128), axis=1))
            rstd = lax.rsqrt(jnp.mean(xc * xc, axis=-1, keepdims=True) + EPS)
            rs = jnp.sum(xc * w2, axis=-1, keepdims=True) * rstd + r0c
            rs = rs.astype(BF).astype(F32)
            mu_b[r0:r0 + n, :] = mu
            rs_b[r0:r0 + n, :] = rstd
            if GC:
                xv = (acc[pl.ds(gated(r0, gate(rstd)), n), :] if not copy else tmp[(r0 % BQ) // 128][pl.ds(gated(r0 % 128, gate(rstd)), n), :])
                xc = xv - (jnp.concatenate([mu] * (D // 128), axis=1))
            out = pk((xv + cb2 + (xv * rstd - jnp.concatenate([mu * rstd] * (D // 128), axis=1)) * ca_).astype(BF))
            ob[r0 // 2:(r0 + n) // 2, :] = out
            if copy:
                acc[r0:r0 + n, :] = xv
            for u in range(n // 8):
                rv = rs[u * 8:(u + 1) * 8]
                idx = lax.broadcasted_iota(I32, (8, 1), 0) + (r0 + u * 8)
                g1_ = rv > m1
                g2_ = rv > m2
                m2 = jnp.where(g1_, m1, jnp.where(g2_, rv, m2))
                i2 = jnp.where(g1_, i1, jnp.where(g2_, idx, i2))
                m1 = jnp.where(g1_, rv, m1)
                i1 = jnp.where(g1_, idx, i1)
            return (m1, i1, m2, i2), out

        ozv = jnp.full((8, 128), pid, I32).astype(U32)

        def after(v, out):
            t = out[:, 0:128]
            for cc in range(1, D // 128):
                t = t | out[:, cc * 128:(cc + 1) * 128]
            return jnp.where((t & ozv) != 0, 0.0, v)

        def done(r0, top):
            t = ob[pl.ds(pl.multiple_of(r0 // 2 + pid * 8, 8), 8), 0:128]
            for v in top:
                t = t ^ pltpu.bitcast(jnp.broadcast_to(v, (8, 128)), U32)
            return pltpu.bitcast(t, I32)[0, 0] & pid

        def attend(h, j, slot):
            do_pv(slot, j, do_qk(h, j))

        cp_c.start()
        cp_x[0].start()
        for cp in cp_m:
            cp.start()
        g0[2].start()
        g0[0].start()
        g0[1].start()
        cp_x[1].start()
        cp_x[2].start()
        cp_x[3].start()
        g0[3].start()
        for cp in g1:
            cp.start()
        for g in range(2, len(GROUPS)):
            for cp in group_copies(g):
                cp.start()
        cp_r.start()
        cp_m2.start()
        for cp in cp_w:
            cp.start()

        def zero(i, carry):
            acc[pl.ds(pl.multiple_of(i * 64, 64), 64), :] = jnp.zeros((64, D), F32)
            return carry
        lax.fori_loop(0, S // 64, zero, 0)
        cp_c.wait()
        cv = cb_[...].astype(F32)
        sc = jnp.broadcast_to(cv * jax.nn.sigmoid(cv), (16, D)).astype(BF)
        cp_x[0].wait()
        for c0 in range(0, BQ, LC):
            tmp[c0 // 128][c0 % 128:c0 % 128 + LC, :] = ln(xb[c0:c0 + LC, :].astype(F32))
        for i, cp in enumerate(cp_m):
            cp.wait()
            mod[:, i * MC:(i + 1) * MC] = jnp.dot(sc, ldw(wm[:, i * MC:(i + 1) * MC]),
                                                  preferred_element_type=F32)[0:8]
        for c0 in range(0, BQ, LC):
            hv = tmp[c0 // 128][c0 % 128:c0 % 128 + LC, :] * (1.0 + mod[0:1, D:2 * D]) + mod[0:1, 0:D]
            hb[hrows(0, c0, LC), :] = pk(hv.astype(BF))
        g0[2].wait()
        do_vt(0, 0)
        g0[0].wait()
        do_qproj(0, 0)

        g0[1].wait()
        for j in range(NT if PEEL0 else 0):
            m = do_qk(0, j)
            if j == 0:
                cp_x[1].wait()
                do_ln1(1)
                for c in range(NQ - 1):
                    do_pv_q(0, 0, c, m)
                do_qproj(0, 1)
                last = do_pv_q(0, 0, NQ - 1, m)
                continue
            if j == 1:
                for cp in (cp_x[2], cp_x[3], g0[3], g1[0]):
                    cp.wait()
            do_oproj(0, j - 1)
            if j + 1 < NT:
                do_ln1(j + 1, gate(last) if j > 1 else None)
                do_qproj(0, j + 1)
            else:
                do_qproj(1, 0)
            last = do_pv(0, j, m)[NQ - 1]
        for cp in g1[1:]:
            cp.wait()

        def body(h, carry):
            for g in range(2, len(GROUPS)):
                @pl.when(h == GROUPS[g][0] - 1)
                def _():
                    for cp in group_copies(g):
                        cp.wait()

            @pl.when(h == MODH)
            def _():
                cp_m2.wait()
                for i in range(2, 6):
                    mod[:, i * D:(i + 1) * D] = jnp.dot(sc, ldw(wm[:, i * D:(i + 1) * D]),
                                                        preferred_element_type=F32)[0:8]
            slot = h % 2
            do_vt(h, slot)
            for j in range(NT):
                m = do_qk(h, j)
                if j > 0:
                    do_oproj(h, j - 1)
                else:
                    do_oproj(h - 1, NT - 1)
                if j + 1 < NT:
                    do_qproj(h, j + 1)
                else:
                    do_qproj(h + 1, 0)
                do_pv(slot, j, m)
            return carry
        lax.fori_loop(1, H - 1, body, 0)

        h = H - 1
        slot = pid + h % 2
        rid8 = lax.broadcasted_iota(I32, (8, 1), 0)
        top = (jnp.full((8, 1), -jnp.inf, F32), rid8, jnp.full((8, 1), -jnp.inf, F32), rid8 + 8)
        h = H - 1
        slot = pid + h % 2
        rid8 = lax.broadcasted_iota(I32, (8, 1), 0)
        top = (jnp.full((8, 1), -jnp.inf, F32), rid8, jnp.full((8, 1), -jnp.inf, F32), rid8 + 8)
        cp_r.wait()
        for cp in cp_w:
            cp.wait()
        consts = epi_consts()
        do_vt(h, slot)
        for j in range(NT if PEEL1 else 0):
            def qk(a, b, z=None):
                ks = slice(a // 2, b // 2) if z is None else pl.ds(pl.multiple_of(a // 2 + z * 8, 8), (b - a) // 2)
                return lax.dot_general(ldw(kb[h, ks, :]), upk(qb[j]), NT_DIMS, preferred_element_type=F32)
            ss = [qk(0, QS1)]
            zs = {}
            if j == 0:
                do_oproj(h - 1, NT - 1)
            else:
                x1, mu = epi_a(h, j - 1, 0, BQ)
                outs = []
                if GB == 2:
                    zb = [gate(mu[c0:c0 + EC]) for c0 in range(0, BQ, EC)]
                elif GB == 3:
                    zb = [gate(mu)] * (BQ // EC)
                for c, c0 in enumerate(range(0, BQ, EC)):
                    r0 = (j - 1) * BQ + c0
                    if GB:
                        xv = acc[pl.ds(gated(r0, gate(mu[c0:c0 + EC]) if GB == 1 else zb[c]), EC), :]
                    else:
                        xv = x1[c0:c0 + EC]
                    if NCH:
                        for u0 in range(0, EC, UR):
                            muu = mu[c0 + u0:c0 + u0 + UR]
                            if len(outs) >= NCH:
                                o_ = outs[-NCH]
                                muu = jnp.concatenate([after(muu[e:e + 8], o_[(e // 2 // 8) * 8:(e // 2 // 8) * 8 + 8]) for e in range(0, UR, 8)], axis=0)
                            top, out = epi_bc(r0 + u0, UR, xv[u0:u0 + UR], muu, top, consts, False)
                            outs.append(out)
                    else:
                        top, _ = epi_bc(r0, EC, xv, mu[c0:c0 + EC], top, consts, False)
                    if DL[c] >= 0:
                        zs[DL[c]] = done(r0, top)
            for p, a in enumerate(range(QS1, S, 256)):
                ss.append(qk(a, a + 256, zs.get(p)))
            s = jnp.concatenate(ss, axis=0)
            m = s, jnp.max(s, axis=0, keepdims=True)
            if j + 1 < NT:
                w = ldw(wqb[:, h * DH:(h + 1) * DH])
                n = BQ // QP
                for p in range(QP):
                    z = zs.get(6 + p)
                    r0 = ((j + 1) * BQ + p * n) // 2
                    rs_ = slice(r0, r0 + n // 2) if z is None else pl.ds(pl.multiple_of(r0 + z * 8, 8), n // 2)
                    q = jnp.dot(upk(hb[rs_, :]), w, preferred_element_type=F32)
                    qb[j + 1, p * n // 2:(p + 1) * n // 2, :] = pk((q * QSCALE).astype(BF))
                do_pv(slot, j, m)
                if j == NT - 2:
                    cp_o[0].start()
                    cp_o[1].start()
            else:
                for c in range(NQ + 1):
                    if c < NQ:
                        do_pv_q(slot, j, c, m)
                    if c > 0:
                        x1, mu = epi_a(h, j, (c - 1) * 128, 128, tmp[c - 1])
                        top, _ = epi_bc(j * BQ + (c - 1) * 128, 128, x1, mu, top, consts, True)
        cp_o[2].start()
        cp_o[3].start()

        m1, i1, m2, i2 = top
        big = jnp.int32(2 * S)
        t1 = jnp.max(m1, axis=0, keepdims=True)
        j1 = jnp.min(jnp.where(m1 == t1, i1, big), axis=0, keepdims=True)
        cm = jnp.where(i1 == j1, m2, m1)
        ci = jnp.where(i1 == j1, i2, i1)
        t2 = jnp.max(cm, axis=0, keepdims=True)
        j2 = jnp.min(jnp.where(cm == t2, ci, big), axis=0, keepdims=True)
        a1 = jnp.clip(j1[0, 0], 0, S - 1)
        a2 = jnp.clip(j2[0, 0], 0, S - 1)
        base1 = pl.multiple_of((a1 // 16) * 16, 16)
        base2 = pl.multiple_of((a2 // 16) * 16, 16)
        rid = lax.broadcasted_iota(I32, (16, D), 0)

        def get_row(a, base):
            r = pl.ds(base, 16)
            t = (acc[r, :] - jnp.concatenate([mu_b[r, :]] * (D // 128), axis=1)) * rs_b[r, :]
            blk = t * (1.0 + mod[0:1, 4 * D:5 * D]) + mod[0:1, 3 * D:4 * D]
            return jnp.sum(jnp.where(rid == a - base, blk, 0.0), axis=0, keepdims=True)
        xs = jnp.where(rid == 0, get_row(a1, base1), jnp.where(rid == 1, get_row(a2, base2), 0.0)).astype(BF)
        g = jnp.dot(xs, ldw(wg[...]), preferred_element_type=F32)
        u = jnp.dot(xs, ldw(wu[...]), preferred_element_type=F32)
        gu = (g * jax.nn.sigmoid(g) * u).astype(BF)
        y = jnp.dot(gu, ldw(wd[...]), preferred_element_type=F32)
        y1 = y[0:1] * jax.nn.sigmoid(jnp.broadcast_to(t1, (1, D)))
        y2 = y[1:2] * jax.nn.sigmoid(jnp.broadcast_to(t2, (1, D)))

        def patch(i, base):
            r = pl.ds(base, 16)
            x1 = acc[r, :]
            row = rid + base
            upd = jnp.where(row == a1, y1, 0.0) + jnp.where(row == a2, y2, 0.0)
            pre = x1 + consts[1] + ((x1 - jnp.concatenate([mu_b[r, :]] * (D // 128), axis=1)) * rs_b[r, :]) * consts[0]
            pb[i] = (pre + mod[0:1, 5 * D:6 * D] * upd).astype(BF)
            return pltpu.make_async_copy(pb.at[i], o_hbm.at[r], sem_s.at[2 + i])
        cp_p1 = patch(0, base1)
        cp_p2 = patch(1, base2)
        for cp in cp_o:
            cp.wait()
        cp_p1.start()

        @pl.when(base1 != base2)
        def _():
            cp_p2.start()
            cp_p2.wait()
        cp_p1.wait()

    any_spec = pl.BlockSpec(memory_space=pl.ANY)

    def wbuf(*shape):
        if PACKW:
            return pltpu.VMEM(shape[:-2] + (shape[-2] // 2, shape[-1]), U32)
        return pltpu.VMEM(shape, BF)
    scratch = [
        pltpu.VMEM((S, D), BF),
        pltpu.VMEM((S // 2, D), U32),
        wbuf(H, S, DH),
        wbuf(H, S, DH),
        wbuf(D, H * DH),
        wbuf(H * DH, D),
        pltpu.VMEM((S, D), F32),
        pltpu.VMEM((NT, BQ // 2, DH), U32),
        pltpu.VMEM((NT, DH // 2, BQ), U32),
        pltpu.VMEM((2, S // 128, 64, 128), U32),
        pltpu.VMEM((128, D), F32), pltpu.VMEM((128, D), F32), pltpu.VMEM((128, D), F32), pltpu.VMEM((128, D), F32),
        pltpu.VMEM((S, 128), F32), pltpu.VMEM((S, 1), F32),
        wbuf(D, F), wbuf(D, F), wbuf(F, D),
        wbuf(D, 6 * D),
        pltpu.VMEM((1, D), BF),
        pltpu.VMEM((1, D), BF),
        pltpu.VMEM((8, 6 * D), F32),
        pltpu.VMEM((S // 2, D), U32),
        pltpu.VMEM((2, 16, D), BF),
        pltpu.SemaphoreType.DMA((4,)),
        pltpu.SemaphoreType.DMA((NT,)),
        pltpu.SemaphoreType.DMA((len(GROUPS), 4)),
        pltpu.SemaphoreType.DMA((5,)),
        pltpu.SemaphoreType.DMA((3,)),
        pltpu.SemaphoreType.DMA((NT,)),
    ]
    call = pl.pallas_call(
        kernel,
        grid=(1,),
        out_shape=jax.ShapeDtypeStruct((S, D), BF),
        in_specs=[any_spec] * 11,
        out_specs=any_spec,
        scratch_shapes=scratch,
        compiler_params=pltpu.CompilerParams(vmem_limit_bytes=124 * 1024 * 1024),
    )

    def kern(A_x, A_k_cache, A_v_cache, A_wq, A_wo, B_x, B_w_r, B_w_gate, B_w_up, B_w_down, c, w_mod):
        out = call(A_x.reshape(S, D), A_k_cache.reshape(H, S, DH), A_v_cache.reshape(H, S, DH), A_wq, A_wo,
                   B_w_r.reshape(1, D), B_w_gate, B_w_up, B_w_down, c, w_mod)
        return out.reshape(1, S, D)
    return kern


_impl = build(NCH=3, EC=128, DL=(4, 6, 8, 9), QP=4)


@jax.jit
def pallas_adaLN_cond__mha_block_cached__moe_arch_mod__prompt_kernel(
        A_x, A_k_cache, A_v_cache, A_wq, A_wo, B_x, B_w_r, B_w_gate, B_w_up, B_w_down, c, w_mod):
    return _impl(A_x, A_k_cache, A_v_cache, A_wq, A_wo, B_x, B_w_r, B_w_gate, B_w_up, B_w_down, c, w_mod)
```

```python
import jax
import jax.numpy as jnp
from jax import lax
import jax.experimental.pallas as pl
import jax.experimental.pallas.tpu as pltpu

S = 2048
D = 1024
H = 32
DH = 128
F = 3584
EPS = 1e-5
BF = jnp.bfloat16
F32 = jnp.float32
U32 = jnp.uint32
I32 = jnp.int32
LOG2E = 1.4426950408889634
QSCALE = (DH ** -0.5) * LOG2E
NT_DIMS = (((1,), (1,)), ((), ()))
TN_DIMS = (((0,), (0,)), ((), ()))

BQ = 512
NT = S // BQ
NQ = BQ // 128
KG = 512
MC = 512
L_LO = 1.0
L_HI = 2.0 ** 60
GROUPS = ((0, 1), (1, 2), (2, 4), (4, 8), (8, 14), (14, H))
WAITH = (None, 0, 0, 2, 6, 12)


def pk(x):
    return pltpu.bitcast(x, U32)


def upk(x):
    return pltpu.bitcast(x, BF)


def lanes(v):
    return jnp.concatenate([v] * (D // 128), axis=1)


def gate(val):
    return jnp.where(val[-8:] < 0.0, 1, 0).astype(I32)[0, 0]


def build(LC=64, EC=128, DL=(9, 11, 13, 15), QP=1, NCH=0, UR=16, QPOS=0, FB=3, LNCH=0, MODH=8, SC=False, BENCH=0,
          FORCE=0, LAG=4, OP=6, QPL=14, EOP=5, SB=1, ST=2, SP=47, CCH=0, RL=0, SS=4, CJ=2, U=1, EU=1):
    def kernel(x_hbm, k_hbm, v_hbm, wq_hbm, wo_hbm, wr_hbm, wg_hbm, wu_hbm, wd_hbm, c_hbm, wmod_hbm,
               o_hbm,
               xb, hb, kb, vb, wqb, wob, acc, qb, ot, vt, tmp0, tmp1, tmp2, tmp3, mu_b, rs_b, topb,
               wg, wu, wd, wm, cb_, wrb, scb, mod, ob, pb,
               sem_s, sem_x, sem_h, sem_m, sem_w, sem_o):
        tmp = (tmp0, tmp1, tmp2, tmp3)
        cur = []

        def mark(name):
            if SC:
                if cur:
                    cur.pop().__exit__(None, None, None)
                if name:
                    cm = jax.named_scope(name)
                    cm.__enter__()
                    cur.append(cm)

        def pw(ref):
            return ref.bitcast(BF)

        def group_copies(g):
            a, b = GROUPS[g]
            return [pltpu.make_async_copy(wq_hbm.at[:, a * DH:b * DH], pw(wqb).at[:, a * DH:b * DH], sem_h.at[g, 0]),
                    pltpu.make_async_copy(k_hbm.at[a:b], pw(kb).at[a:b], sem_h.at[g, 1]),
                    pltpu.make_async_copy(v_hbm.at[a:b], pw(vb).at[a:b], sem_h.at[g, 2]),
                    pltpu.make_async_copy(wo_hbm.at[a * DH:b * DH, :], pw(wob).at[a * DH:b * DH, :], sem_h.at[g, 3])]

        def x_copy(r0, i):
            return pltpu.make_async_copy(x_hbm.at[pl.ds(r0, BQ)], xb.at[pl.ds(r0, BQ)], sem_x.at[i])
        cp_c = pltpu.make_async_copy(c_hbm, cb_, sem_s.at[0])
        cp_r = pltpu.make_async_copy(wr_hbm, wrb, sem_s.at[1])
        cp_x = [x_copy(j * BQ, j) for j in range(NT)]
        cp_m = [pltpu.make_async_copy(wmod_hbm.at[:, i * MC:(i + 1) * MC], pw(wm).at[:, i * MC:(i + 1) * MC],
                                      sem_m.at[i]) for i in range(2 * D // MC)]
        cp_m2 = pltpu.make_async_copy(wmod_hbm.at[:, 2 * D:], pw(wm).at[:, 2 * D:], sem_m.at[2 * D // MC])
        cp_w = [pltpu.make_async_copy(wg_hbm, pw(wg), sem_w.at[0]),
                pltpu.make_async_copy(wu_hbm, pw(wu), sem_w.at[1]),
                pltpu.make_async_copy(wd_hbm, pw(wd), sem_w.at[2])]
        cp_o = [pltpu.make_async_copy(pw(ob).at[j * BQ:(j + 1) * BQ], o_hbm.at[j * BQ:(j + 1) * BQ], sem_o.at[j])
                for j in range(NT)]
        g0 = group_copies(0)
        g1 = group_copies(1)

        def rows(j, lo=0, n=BQ, half=False):
            k = 2 if half else 1
            if isinstance(j, int):
                return pl.ds((j * BQ + lo) // k, n // k)
            return pl.ds(pl.multiple_of(j * (BQ // k) + lo // k, 8), n // k)

        def ln(xf):
            xc = xf - jnp.mean(xf, axis=-1, keepdims=True)
            return xc * lax.rsqrt(jnp.mean(xc * xc, axis=-1, keepdims=True) + EPS)

        def do_ln1(j):
            for c0 in range(0, BQ, LC):
                hv = ln(xb[rows(j, c0, LC), :].astype(F32)) * (1.0 + mod[0:1, D:2 * D]) + mod[0:1, 0:D]
                hb[rows(j, c0, LC, True), :] = pk(hv.astype(BF))

        def do_qproj(h, j, slot):
            w = upk(wqb[:, h * DH:(h + 1) * DH] if isinstance(h, int)
                    else wqb[:, pl.ds(pl.multiple_of(h * DH, DH), DH)])
            q = jnp.dot(upk(hb[rows(j, half=True), :]), w, preferred_element_type=F32)
            qb[slot] = pk((q * QSCALE).astype(BF))

        def scores(h, slot, ks=slice(None)):
            return lax.dot_general(upk(kb[h, ks, :]), upk(qb[slot]), NT_DIMS, preferred_element_type=F32)

        def wo_of(h):
            return upk(wob[pl.ds(pl.multiple_of(h * (DH // 2), DH // 2), DH // 2), :])

        def do_oproj(h, j):
            acc[rows(j), :] += lax.dot_general(upk(ot[j]), wo_of(h), TN_DIMS, preferred_element_type=F32)

        def do_vt(h, slot):
            for i in range(S // 128):
                vt[slot, i] = pk(upk(vb[h, i * 64:(i + 1) * 64, :]).T)

        def do_pv_q(slot, jj, c, s, m, bad):
            o = l = None
            for g in range(S // KG):
                p = s[g * KG:(g + 1) * KG, c * 128:(c + 1) * 128]
                if m is not None:
                    p = p - m[:, c * 128:(c + 1) * 128]
                p = jnp.exp2(p)
                ls = jnp.sum(p, axis=0, keepdims=True)
                l = ls if l is None else l + ls
                lhs = jnp.concatenate([upk(vt[slot, g * (KG // 128) + u]) for u in range(KG // 128)], axis=1)
                d = jnp.dot(lhs, p.astype(BF), preferred_element_type=F32)
                o = d if o is None else o + d
            ot[jj, :, c * 128:(c + 1) * 128] = pk((o * (1.0 / l)).astype(BF))
            if m is None:
                return jnp.where((l > L_LO) & (l < L_HI), bad, 1.0)
            return bad

        def do_pv(slot, jj, s, m, bad):
            for c in range(NQ):
                bad = do_pv_q(slot, jj, c, s, m, bad)
            return bad

        def attend(h, slot, tiles, bad, hooks):
            NG = S // KG
            N = len(tiles) * NQ * NG
            P = {}
            st = {}
            for n in range(N + LAG):
                if n < N:
                    j, c, g = tiles[n // (NQ * NG)], n // NG % NQ, n % NG
                    z = hooks.get(('z', n))
                    kr = pl.ds(g * (KG // 2), KG // 2) if z is None else pl.ds(pl.multiple_of(g * (KG // 2) + z * 8, 8), KG // 2)
                    s = lax.dot_general(upk(kb[h, kr, :]), upk(qb[j, c * 64:(c + 1) * 64, :]), NT_DIMS,
                                        preferred_element_type=F32)
                    P[n] = jnp.exp2(s)
                for fn in hooks.get(n, ()):
                    fn()
                k = n - LAG
                if k >= 0:
                    j, c, g = tiles[k // (NQ * NG)], k // NG % NQ, k % NG
                    p = P.pop(k)
                    ls = jnp.sum(p, axis=0, keepdims=True)
                    lhs = jnp.concatenate([upk(vt[slot, g * (KG // 128) + u]) for u in range(KG // 128)], axis=1)
                    d = jnp.dot(lhs, p.astype(BF), preferred_element_type=F32)
                    st['l'] = ls if g == 0 else st['l'] + ls
                    st['o'] = d if g == 0 else st['o'] + d
                    if g == NG - 1:
                        l = st['l']
                        ot[j, :, c * 128:(c + 1) * 128] = pk((st['o'] * (1.0 / l)).astype(BF))
                        bad = jnp.where((l > L_LO) & (l < L_HI), bad, 1.0)
                        for fn in hooks.get(('o', k), ()):
                            fn()
            return bad

        TS = NQ * (S // KG)

        def fast_head(h, bad):
            slot = h % 2
            do_vt(h, slot)
            hooks = {}
            for j in range(NT):
                hooks[j * TS + QPOS] = [lambda j=j: do_qproj(h + (j + 1) // NT, (j + 1) % NT, (j + 1) % NT)]
                hooks.setdefault(j * TS + OP, []).append(lambda j=j: do_oproj(jnp.where(h == 0, H, h - 1) if j == 0 else h, (j - 1) % NT))
            return attend(h, slot, list(range(NT)), bad, hooks)

        def epi_consts():
            cb1 = 1.0 + mod[0:1, 4 * D:5 * D]
            sbv = mod[0:1, 3 * D:4 * D]
            gb = mod[0:1, 5 * D:6 * D]
            wr = wrb[...].astype(F32).reshape(1, D)
            return gb * cb1, gb * sbv, wr * cb1, jnp.sum(wr * sbv, axis=-1, keepdims=True)

        def row_mean(x1):
            return jnp.broadcast_to(jnp.mean(x1, axis=-1, keepdims=True), (x1.shape[0], 128))

        def epi_a(h, j, lo, n, buf=None):
            rr = rows(j, lo, n)
            d = lax.dot_general(upk(ot[j, :, lo:lo + n]), wo_of(h), TN_DIMS, preferred_element_type=F32)
            x1 = xb[rr, :].astype(F32) + mod[0:1, 2 * D:3 * D] * (acc[rr, :] + d)
            if buf is None:
                acc[rr, :] = x1
            else:
                buf[...] = x1
            return x1, row_mean(x1)

        def epi_bc(r0, n, xv, mu, top, consts, copy, noc=False):
            m1, i1, m2, i2, bad = top
            ca_, cb2, w2, r0c = consts
            xc = xv - lanes(mu)
            rstd = lax.rsqrt(jnp.mean(xc * xc, axis=-1, keepdims=True) + EPS)
            rs = jnp.sum(xc * w2, axis=-1, keepdims=True) * rstd + r0c
            rs = rs.astype(BF).astype(F32)
            rr = pl.ds(r0, n)
            mu_b[rr, :] = mu
            rs_b[rr, :] = jnp.broadcast_to(rstd, (n, 128))
            hr = pl.ds(r0 // 2 if isinstance(r0, int) else pl.multiple_of(r0 // 2, 8), n // 2)
            out = pk((xv + cb2 + (xv * rstd - lanes(mu * rstd)) * ca_).astype(BF))
            if not noc:
                ob[hr, :] = out
            if copy:
                acc[rr, :] = xv
            for u in range(n // 8):
                rv = rs[u * 8:(u + 1) * 8]
                idx = lax.broadcasted_iota(I32, (8, 1), 0) + (r0 + u * 8)
                g1_ = rv > m1
                g2_ = rv > m2
                m2 = jnp.where(g1_, m1, jnp.where(g2_, rv, m2))
                i2 = jnp.where(g1_, i1, jnp.where(g2_, idx, i2))
                m1 = jnp.where(g1_, rv, m1)
                i1 = jnp.where(g1_, idx, i1)
                bad = jnp.where(rv == rv, bad, 1.0)
            return (m1, i1, m2, i2, bad), out

        def top_init():
            rid8 = lax.broadcasted_iota(I32, (8, 1), 0)
            return (jnp.full((8, 1), -jnp.inf, F32), rid8, jnp.full((8, 1), -jnp.inf, F32), rid8 + 8,
                    jnp.zeros((8, 1), F32))

        def top_store(top):
            for i, v in enumerate(top[:4]):
                topb[i] = jnp.broadcast_to(pltpu.bitcast(v, I32), (8, 128))

        def zero_acc():
            def zero(i, carry):
                acc[pl.ds(pl.multiple_of(i * 64, 64), 64), :] = jnp.zeros((64, D), F32)
                return carry
            lax.fori_loop(0, S // 64, zero, 0)
            ot[NT - 1] = jnp.zeros((DH // 2, BQ), U32)

        def do_mod(lo, n):
            return jnp.dot(scb[...], upk(wm[:, pl.ds(lo, n)]), preferred_element_type=F32)[0:8]

        if BENCH:
            def bbody(i, bad):
                return fast_head(1 + (i & 15), bad)
            bad = lax.fori_loop(0, BENCH, bbody, jnp.zeros((1, 128), F32))
            topb[0] = jnp.broadcast_to(pltpu.bitcast(bad, I32), (8, 128))
            cp = pltpu.make_async_copy(pw(ob), o_hbm, sem_o.at[0])
            cp.start()
            cp.wait()
            return

        mark('s0')
        cp_c.start()
        for cp in cp_m:
            cp.start()
        cp_x[0].start()
        zero_acc()
        wob[H * (DH // 2):, :] = jnp.zeros((DH // 2, D), U32)
        cp_c.wait()
        cv = cb_[...].astype(F32)
        scb[...] = jnp.broadcast_to(cv * jax.nn.sigmoid(cv), (16, D)).astype(BF)
        mark('s1')

        def mod_body(i, carry):
            pltpu.make_async_copy(
                wmod_hbm.at[:, 0:MC], pw(wm).at[:, 0:MC], sem_m.at[i]).wait()

            @pl.when(i == ST)
            def _():
                for c2 in cp_x[1:] + [g0[1], g0[2], g0[0], g0[3], g1[0]]:
                    c2.start()
            lo = pl.multiple_of(i * MC, MC)
            mod[:, pl.ds(lo, MC)] = do_mod(lo, MC)
            return carry
        lax.fori_loop(0, 2 * D // MC, mod_body, 0)
        mark('s2')

        def ln_body(j, carry):
            x_copy(pl.multiple_of(j * BQ, BQ), j).wait()
            do_ln1(j)
            return carry
        lax.fori_loop(0, NT, ln_body, 0)
        mark('s3')
        for cp in g0 + [g1[0]]:
            cp.wait()
        for cp in g1[1:]:
            cp.start()
        for g in range(2, len(GROUPS)):
            for cp in group_copies(g):
                cp.start()
        for cp in [cp_r, cp_m2] + cp_w:
            cp.start()
        do_qproj(0, 0, 0)

        def safe_attention():
            cp_o[0].wait()
            cp_o[1].wait()
            zero_acc()

            def hbody(h, carry):
                do_vt(h, 0)

                def unit(u, carry):
                    q = jnp.dot(upk(hb[pl.ds(pl.multiple_of(u * 64, 64), 64), :]),
                                upk(wqb[:, pl.ds(pl.multiple_of(h * DH, DH), DH)]), preferred_element_type=F32)
                    q = (q * QSCALE).astype(BF)

                    def sc(g):
                        return lax.dot_general(upk(kb[h, pl.ds(pl.multiple_of(g * (KG // 2), KG // 2), KG // 2), :]),
                                               q, NT_DIMS, preferred_element_type=F32)
                    m = lax.fori_loop(0, S // KG, lambda g, m: jnp.maximum(m, jnp.max(sc(g), axis=0, keepdims=True)),
                                      jnp.full((1, 128), -jnp.inf, F32))

                    def pv(g, c):
                        p = jnp.exp2(sc(g) - m)
                        lhs = jnp.concatenate([upk(vt[0, g * (KG // 128) + i]) for i in range(KG // 128)], axis=1)
                        return (c[0] + jnp.dot(lhs, p.astype(BF), preferred_element_type=F32),
                                c[1] + jnp.sum(p, axis=0, keepdims=True))
                    o, l = lax.fori_loop(0, S // KG, pv, (jnp.zeros((DH, 128), F32), jnp.zeros((1, 128), F32)))
                    o = (o * (1.0 / l)).astype(BF)
                    r = pl.ds(pl.multiple_of(u * 128, 128), 128)
                    acc[r, :] += lax.dot_general(o, wo_of(h), TN_DIMS, preferred_element_type=F32)
                    return carry
                lax.fori_loop(0, S // 128, unit, 0)
                return carry
            lax.fori_loop(0, H, hbody, 0)
            consts = epi_consts()

            def ebody(i, top):
                r0 = pl.multiple_of(i * 64, 64)
                x1 = xb[pl.ds(r0, 64), :].astype(F32) + mod[0:1, 2 * D:3 * D] * acc[pl.ds(r0, 64), :]
                return epi_bc(r0, 64, x1, row_mean(x1), top, consts, True)[0]
            top_store(lax.fori_loop(0, S // 64, ebody, top_init()))
            cp_o[0].start()
            cp_o[1].start()

        def head_body(i, bad):
            for uu in range(U):
                bad = one(i * U + uu, bad, uu == 0)
            return bad

        def one(h, bad, lead):
            if not lead:
                return fast_head(h, bad)
            for g in range(1, len(GROUPS)):
                @pl.when(h == (WAITH[g] if U > 1 or g > 2 else 1))
                def _():
                    for cp in (g1[1:] if g == 1 else group_copies(g)):
                        cp.wait()

            @pl.when(h == MODH)
            def _():
                cp_m2.wait()

                def mbody(i, carry):
                    lo = pl.multiple_of(i * D, D)
                    mod[:, pl.ds(lo, D)] = do_mod(lo, D)
                    return carry
                lax.fori_loop(2, 6, mbody, 0)
            return fast_head(h, bad)
        mark('s5')
        bad = lax.fori_loop(0, H // U if U > 1 else H - 1, head_body, jnp.zeros((1, 128), F32))

        def fast_rest():
            nonlocal bad
            mark('s6')
            cp_r.wait()
            for cp in cp_w:
                cp.wait()
            if U > 1:
                consts = epi_consts()
                top = top_init()
                for c in range(NQ):
                    x1, mu = epi_a(H - 1, NT - 1, c * 128, 128, tmp[c])
                    top, _ = epi_bc((NT - 1) * BQ + c * 128, 128, x1, mu, top, consts, True, True)

                def ebody(i, top):
                    r0 = pl.multiple_of(i * 128, 128)
                    x1 = xb[pl.ds(r0, 128), :].astype(F32) + mod[0:1, 2 * D:3 * D] * acc[pl.ds(r0, 128), :]
                    return epi_bc(r0, 128, x1, row_mean(x1), top, consts, True)[0]
                top = lax.fori_loop(0, (NT - 1) * NQ, ebody, top, unroll=EU)
                cp_o[0].start()
                cp_o[1].start()
                return top, bad
            h = H - 1
            pid = gate(jnp.exp2(mod[0:8, 0:128]))
            pid2 = gate(jnp.exp2(mod[0:8, 128:256]))
            ozv = jnp.full((8, 128), pid, I32).astype(U32)
            slot = pid + h % 2
            top = top_init()
            consts = epi_consts()

            def gated(base, z, al):
                return base if z is None else pl.multiple_of(base + z * al, al)

            def after(v, out):
                t = out[:, 0:128]
                for cc in range(1, D // 128):
                    t = t | out[:, cc * 128:(cc + 1) * 128]
                return jnp.where((t & ozv) != 0, 0.0, v)

            def done(r0, top):
                t = ob[pl.ds(pl.multiple_of(r0 // 2 + pid * 8, 8), 8), 0:128]
                for v in top:
                    t = t ^ pltpu.bitcast(jnp.broadcast_to(v, (8, 128)), U32)
                return pltpu.bitcast(t, I32)[0, 0] & pid

            do_vt(h, slot)
            state = {'top': top}
            hooks = {}

            def epi(j, n0):
                x1, mu = epi_a(h, j, 0, BQ)
                top = state['top']
                outs = []
                for c, c0 in enumerate(range(0, BQ, EC)):
                    if NCH:
                        for u0 in range(c0, c0 + EC, UR):
                            muu = mu[u0:u0 + UR]
                            if len(outs) >= NCH:
                                muu = jnp.concatenate(
                                    [after(muu[e:e + 8], outs[-NCH][e // 16 * 8:e // 16 * 8 + 8])
                                     for e in range(0, UR, 8)], axis=0)
                            top, out = epi_bc(j * BQ + u0, UR, acc[pl.ds(pl.multiple_of(j * BQ + u0 + pid * 8, 8), UR), :] if RL else x1[u0:u0 + UR], muu, top, consts, False)
                            outs.append(out)
                    else:
                        top, _ = epi_bc(j * BQ + c0, EC, x1[c0:c0 + EC], mu[c0:c0 + EC], top, consts, False)
                    if DL[c] >= 0:
                        hooks[('z', n0 + DL[c])] = done(j * BQ + c0, top)
                state['top'] = top

            def epi2(j, n0):
                x1, mu = epi_a(h, j, 0, BQ)
                m1, i1, m2, i2, bd = state['top']
                ca_, cb2, w2, r0c = consts
                rst, outs = [], []
                for u in range(BQ // 8):
                    r0 = j * BQ + u * 8
                    muu = mu[u * 8:u * 8 + 8]
                    if u >= NCH:
                        muu = jnp.where(rst[u - NCH] < 0.0, 0.0, muu)
                    xc = (acc[pl.ds(pl.multiple_of(r0 + pid * 8, 8), 8), :] if RL else x1[u * 8:u * 8 + 8]) - lanes(muu)
                    rstd = jnp.broadcast_to(lax.rsqrt(jnp.mean(xc * xc, axis=-1, keepdims=True) + EPS), (8, 128))
                    rst.append(rstd)
                    rv = (jnp.sum(xc * w2, axis=-1, keepdims=True) * rstd[:, 0:1] + r0c).astype(BF).astype(F32)
                    mu_b[r0:r0 + 8, :] = muu
                    rs_b[r0:r0 + 8, :] = rstd
                    idx = lax.broadcasted_iota(I32, (8, 1), 0) + r0
                    g1_ = rv > m1
                    g2_ = rv > m2
                    m2 = jnp.where(g1_, m1, jnp.where(g2_, rv, m2))
                    i2 = jnp.where(g1_, i1, jnp.where(g2_, idx, i2))
                    m1 = jnp.where(g1_, rv, m1)
                    i1 = jnp.where(g1_, idx, i1)
                    mr = muu * rstd
                    if u >= CCH:
                        t = outs[u - CCH]
                        w = 1024
                        while w > 128:
                            w //= 2
                            t = jnp.maximum(t[:, :w], t[:, w:])
                        t = jnp.where((pltpu.bitcast(t, U32) & ozv) != 0, 0.0, 1.0)
                        rstd = rstd * t
                    xv = acc[pl.ds(pl.multiple_of(r0 + pid2 * 8, 8), 8), :] if RL else x1[u * 8:u * 8 + 8]
                    ov = xv + cb2 + (xv * lanes(rstd) - lanes(mr)) * ca_
                    outs.append(ov)
                    if u % 2 and j < CJ:
                        ob[r0 // 2 - 4:r0 // 2 + 4, :] = pk(jnp.concatenate(outs[-2:], axis=0).astype(BF))
                state['top'] = (m1, i1, m2, i2, bd)
            if CCH:
                epi = epi2

            def epi_last(c):
                x1, mu = epi_a(h, NT - 1, c * 128, 128, tmp[c])
                state['top'], _ = epi_bc((NT - 1) * BQ + c * 128, 128, x1, mu, state['top'], consts, True, CJ < NT)

            def send():
                cp_o[0].start()
                cp_o[1].start()
            for j in range(NT):
                if j + 1 < NT:
                    hooks[j * TS + QPL] = [lambda j=j: do_qproj(h, j + 1, j + 1)]
                if j == 0:
                    hooks.setdefault(OP, []).append(lambda: do_oproj(h - 1, NT - 1))
                else:
                    hooks.setdefault(j * TS + EOP, []).append(lambda j=j: epi(j - 1, j * TS))
            hooks.setdefault(SP, []).append(send)
            for c in range(NQ - 1):
                hooks.setdefault(min((NT - 1) * TS + SB + c * SS + 4 + LAG + 1, NT * TS + LAG - 1), []).append(lambda c=c: epi_last(c))
            bad = attend(h, slot, list(range(NT)), bad, hooks)
            epi_last(NQ - 1)
            top = state['top']
            mark(None)
            return top, bad

        mark('s4e')
        top, bad = fast_rest()
        top_store(top)

        @pl.when(jnp.max(jnp.maximum(jnp.max(bad, axis=1, keepdims=True), jnp.max(top[4], axis=0, keepdims=True))) + FORCE > 0.5)
        def _():
            safe_attention()

        mark('s7')
        if CJ == NT:
            cp_o[2].start()
            cp_o[3].start()
        m1, m2 = (pltpu.bitcast(topb[i], F32) for i in (0, 2))
        i1, i2 = topb[1], topb[3]
        big = jnp.int32(2 * S)
        t1 = jnp.max(m1, axis=0, keepdims=True)
        j1 = jnp.min(jnp.where(m1 == t1, i1, big), axis=0, keepdims=True)
        cm = jnp.where(i1 == j1, m2, m1)
        ci = jnp.where(i1 == j1, i2, i1)
        t2 = jnp.max(cm, axis=0, keepdims=True)
        j2 = jnp.min(jnp.where(cm == t2, ci, big), axis=0, keepdims=True)
        a1 = jnp.clip(j1[0, 0], 0, S - 1)
        a2 = jnp.clip(j2[0, 0], 0, S - 1)
        base1 = pl.multiple_of((a1 // 16) * 16, 16)
        base2 = pl.multiple_of((a2 // 16) * 16, 16)
        rid = lax.broadcasted_iota(I32, (16, D), 0)
        consts = epi_consts()
        gb = mod[0:1, 5 * D:6 * D]

        def get_row(a, base):
            r = pl.ds(base, 16)
            t = (acc[r, :] - lanes(mu_b[r, :])) * lanes(rs_b[r, :])
            blk = t * (1.0 + mod[0:1, 4 * D:5 * D]) + mod[0:1, 3 * D:4 * D]
            return jnp.sum(jnp.where(rid == a - base, blk, 0.0), axis=0, keepdims=True)
        xs = jnp.where(rid == 0, get_row(a1, base1), jnp.where(rid == 1, get_row(a2, base2), 0.0)).astype(BF)
        g = jnp.dot(xs, upk(wg[...]), preferred_element_type=F32)
        if CJ < NT:
            for r0 in range(CJ * BQ, S, 64):
                xv = acc[r0:r0 + 64, :]
                rstd = rs_b[r0:r0 + 64, :]
                ob[r0 // 2:r0 // 2 + 32, :] = pk(
                    (xv + consts[1] + (xv * lanes(rstd) - lanes(mu_b[r0:r0 + 64, :] * rstd)) * consts[0]).astype(BF))
            cp_o[2].start()
            cp_o[3].start()
        u = jnp.dot(xs, upk(wu[...]), preferred_element_type=F32)
        gu = (g * jax.nn.sigmoid(g) * u).astype(BF)
        y = jnp.dot(gu, upk(wd[...]), preferred_element_type=F32)
        y1 = y[0:1] * jax.nn.sigmoid(lanes(t1))
        y2 = y[1:2] * jax.nn.sigmoid(lanes(t2))
        mark('s8')

        def patch(i, base):
            r = pl.ds(base, 16)
            x1 = acc[r, :]
            row = rid + base
            upd = jnp.where(row == a1, y1, 0.0) + jnp.where(row == a2, y2, 0.0)
            pre = x1 + consts[1] + ((x1 - lanes(mu_b[r, :])) * lanes(rs_b[r, :])) * consts[0]
            pb[i] = (pre + gb * upd).astype(BF)
            return pltpu.make_async_copy(pb.at[i], o_hbm.at[r], sem_s.at[2 + i])
        cp_p1 = patch(0, base1)
        cp_p2 = patch(1, base2)
        for cp in cp_o:
            cp.wait()
        cp_p1.start()

        @pl.when(base1 != base2)
        def _():
            cp_p2.start()
            cp_p2.wait()
        cp_p1.wait()
        mark(None)

    def wbuf(*shape):
        return pltpu.VMEM(shape[:-2] + (shape[-2] // 2, shape[-1]), U32)
    scratch = [
        pltpu.VMEM((S, D), BF),
        wbuf(S, D),
        wbuf(H, S, DH),
        wbuf(H, S, DH),
        wbuf(D, H * DH),
        wbuf((H + 1) * DH, D),
        pltpu.VMEM((S, D), F32),
        wbuf(NT, BQ, DH),
        wbuf(NT, DH, BQ),
        wbuf(2, S // 128, 128, 128),
        pltpu.VMEM((128, D), F32), pltpu.VMEM((128, D), F32), pltpu.VMEM((128, D), F32), pltpu.VMEM((128, D), F32),
        pltpu.VMEM((S, 128), F32), pltpu.VMEM((S, 128), F32),
        pltpu.VMEM((4, 8, 128), I32),
        wbuf(D, F), wbuf(D, F), wbuf(F, D),
        wbuf(D, 6 * D),
        pltpu.VMEM((1, D), BF),
        pltpu.VMEM((D,), BF),
        pltpu.VMEM((16, D), BF),
        pltpu.VMEM((8, 6 * D), F32),
        wbuf(S, D),
        pltpu.VMEM((2, 16, D), BF),
        pltpu.SemaphoreType.DMA((4,)),
        pltpu.SemaphoreType.DMA((NT,)),
        pltpu.SemaphoreType.DMA((len(GROUPS), 4)),
        pltpu.SemaphoreType.DMA((5,)),
        pltpu.SemaphoreType.DMA((3,)),
        pltpu.SemaphoreType.DMA((NT,)),
    ]
    call = pl.pallas_call(
        kernel,
        grid=(1,),
        out_shape=jax.ShapeDtypeStruct((S, D), BF),
        in_specs=[pl.BlockSpec(memory_space=pl.ANY)] * 11,
        out_specs=pl.BlockSpec(memory_space=pl.ANY),
        scratch_shapes=scratch,
        compiler_params=pltpu.CompilerParams(vmem_limit_bytes=124 * 1024 * 1024),
    )

    def kern(A_x, A_k_cache, A_v_cache, A_wq, A_wo, B_x, B_w_r, B_w_gate, B_w_up, B_w_down, c, w_mod):
        out = call(A_x.reshape(S, D), A_k_cache.reshape(H, S, DH), A_v_cache.reshape(H, S, DH), A_wq, A_wo,
                   B_w_r, B_w_gate, B_w_up, B_w_down, c, w_mod)
        return out.reshape(1, S, D)
    return kern


_impl = build(CJ=4, MODH=24, SB=3, EOP=4, QPL=7, SP=50)


@jax.jit
def pallas_adaLN_cond__mha_block_cached__moe_arch_mod__prompt_kernel(
        A_x, A_k_cache, A_v_cache, A_wq, A_wo, B_x, B_w_r, B_w_gate, B_w_up, B_w_down, c, w_mod):
    return _impl(A_x, A_k_cache, A_v_cache, A_wq, A_wo, B_x, B_w_r, B_w_gate, B_w_up, B_w_down, c, w_mod)
```
